```python
import jax
import jax.numpy as jnp

def _softmax(x, axis=-1):
    return jax.nn.softmax(x, axis=axis)
def _gelu(x):
    return jax.nn.gelu(x, approximate=True)
def _silu(x):
    return jax.nn.silu(x)
def _sigmoid(x):
    return jax.nn.sigmoid(x)
def _layernorm(x, axis=-1, eps=1e-5):
    m = jnp.mean(x, axis=axis, keepdims=True)
    v = jnp.var(x, axis=axis, keepdims=True)
    return (x - m) / jnp.sqrt(v + eps)
def _scatter_add(tgt, idx, src, axis=0):
    return tgt.at[idx].add(src)
def _segment_sum(src, seg, n):
    return jax.ops.segment_sum(src, seg, n)
class _Rng:
    def __init__(self, key):
        self._k = key
    def _next(self):
        self._k, sub = jax.random.split(self._k)
        return sub
    def normal(self, shape):
        return jax.random.normal(self._next(), shape, dtype=jnp.bfloat16)
    def randint(self, lo, hi, shape):
        return jax.random.randint(self._next(), shape, lo, hi, dtype=jnp.int32)
    def uniform(self, shape, lo=0.0, hi=1.0):
        return jax.random.uniform(self._next(), shape, jnp.bfloat16, lo, hi)
    def permutation(self, n):
        return jax.random.permutation(self._next(), n)


kernel_name = 'concat_heads__gqa_block_cached__compressed_kv_cla__decode'

def setup_inputs():
    _rng = _Rng(jax.random.key(int.from_bytes(__import__("os").urandom(4), "little")))
    _w = (lambda a: (lambda t: t.astype(jnp.bfloat16) if jnp.issubdtype(t.dtype, jnp.floating) else t)(jnp.asarray(a)))
    def _A_setup():
        B, Sq, D = 2, 1, 512
        Hq, Hkv, Sk, Dh = 32, 32, 8192, 128
        assert Hq % Hkv == 0, (Hq, Hkv)
        return {
            "x": _w((lambda *s: _rng.normal(s) * 0.05)(B, Sq, D)),
            "k_cache": _w((lambda *s: _rng.normal(s) * 0.05)(B, Hkv, Sk, Dh)),
            "v_cache": _w((lambda *s: _rng.normal(s) * 0.05)(B, Hkv, Sk, Dh)),
            "wq": _w((lambda *s: _rng.normal(s) * 0.05)(D, Hq * Dh) * (D ** -0.5)),
            "wo": _w((lambda *s: _rng.normal(s) * 0.05)(Hq * Dh, D) * ((Hq * Dh) ** -0.5)),
        }
    _A_in = _A_setup()

    def _B_setup():
        B, H, Sq, Sk, D, M = 2, 32, 1, 8192, 128, 512
        Dc = 4 * D
        return {
            "x": _w((lambda *s: _rng.normal(s) * 0.05)(B, Sq, M)),
            "c_kv": _w((lambda *s: _rng.normal(s) * 0.05)(B, Sk, Dc)),
            "w_q": _w((lambda *s: _rng.normal(s) * 0.05)(M, H, D) * (M ** -0.5)),
            "w_uk": _w((lambda *s: _rng.normal(s) * 0.05)(Dc, H, D) * (Dc ** -0.5)),
            "w_uv": _w((lambda *s: _rng.normal(s) * 0.05)(Dc, H, D) * (Dc ** -0.5)),
            "w_o": _w((lambda *s: _rng.normal(s) * 0.05)(H, D, M) * ((H * D) ** -0.5)),
        }
    _B_in = _B_setup()

    return {
        "A_x": _A_in["x"],
        "A_k_cache": _A_in["k_cache"],
        "A_v_cache": _A_in["v_cache"],
        "A_wq": _A_in["wq"],
        "A_wo": _A_in["wo"],
        "B_x": _B_in["x"],
        "B_c_kv": _B_in["c_kv"],
        "B_w_q": _B_in["w_q"],
        "B_w_uk": _B_in["w_uk"],
        "B_w_uv": _B_in["w_uv"],
        "B_w_o": _B_in["w_o"],
    }

def reference(A_x, A_k_cache, A_v_cache, A_wq, A_wo, B_x, B_c_kv, B_w_q, B_w_uk, B_w_uv, B_w_o):
    def _A_ref(x, k_cache, v_cache, wq, wo):
        B, Sq, D = x.shape
        Hq, Dh = 32, 128
        Hkv = k_cache.shape[1]
        rep = Hq // Hkv
        q = (lambda x, *d: x.transpose(*d))((x @ wq).reshape(B, Sq, Hq, Dh), 0, 2, 1, 3)
        k = jnp.repeat(k_cache, rep, axis=1)
        v = jnp.repeat(v_cache, rep, axis=1)
        scores = jnp.einsum("bhqd,bhkd->bhqk", q, k) * (Dh ** -0.5)
        p = _softmax(scores, axis=-1)
        o = jnp.einsum("bhqk,bhkd->bhqd", p, v)
        return (lambda x, *d: x.transpose(*d))(o, 0, 2, 1, 3).reshape(B, Sq, Hq * Dh) @ wo

    def _B_ref(x, c_kv, w_q, w_uk, w_uv, w_o):
        B, Sq, M = x.shape[0], x.shape[1], x.shape[2]
        Sk = c_kv.shape[1]
        H, D = w_q.shape[1], w_q.shape[2]
        q = jnp.einsum("bqm,mhd->bhqd", x, w_q)
        k = jnp.einsum("bkc,chd->bhkd", c_kv, w_uk)
        v = jnp.einsum("bkc,chd->bhkd", c_kv, w_uv)
        scores = jnp.einsum("bhqd,bhkd->bhqk", q, k) * (D ** -0.5)
        off = Sk - Sq
        qi = jnp.arange(Sq)[:, None]
        kj = jnp.arange(Sk)[None, :]
        cmask = kj <= (qi + off)
        scores = jnp.where(cmask[None, None], scores, -1e9)
        p = _softmax(scores, axis=-1)
        ctx = jnp.einsum("bhqk,bhkd->bhqd", p, v)
        return jnp.einsum("bhqd,hdm->bqm", ctx, w_o)

    a = _A_ref(A_x, A_k_cache, A_v_cache, A_wq, A_wo)
    b = _B_ref(B_x, B_c_kv, B_w_q, B_w_uk, B_w_uv, B_w_o)
    return jnp.concatenate([a, b], axis=-1)
```

```python
import functools
import numpy as np
import jax
import jax.numpy as jnp
from jax import lax
from jax.experimental import pallas as pl
from jax.experimental.pallas import tpu as pltpu

F32 = jnp.float32
BF16 = jnp.bfloat16
NT = (((1,), (1,)), ((), ()))

NB, NH, SK, DH = 2, 32, 8192, 128
DM = 512
DC = 512
G = 8
NG = NB * NH // G
SCALE = float(DH) ** -0.5


def build(R=256, DR=128, NS=3, RC=512, vmem_mb=100, dma_only=False, side_on=True):
    NC = SK // R
    ND = R // DR
    LA = NS - 1
    TOT = NG * NC
    SIDE = 128
    HALF = NC // 2
    SPS = SIDE // HALF
    NCH = SK // RC
    assert SPS * HALF == SIDE

    def kernel(xa_hbm, k_hbm, v_hbm, wq_hbm, wo_hbm, xb_hbm, c_hbm, wqb_hbm, wuk_hbm, wuv_hbm, wob_hbm,
               out_ref,
               xa_v, xb_v, wq_v, wo_v, c_v, wqb_v, wuk_v, wuv_v, wob_v, kbuf, vbuf,
               qb_s, qabs_s, mb_s, lb_s, accb_s, ctx_s, outb_s,
               kv_sem, misc_sem):
        S_XA, S_XB, S_WQ, S_WO, S_WQB, S_WUK, S_WUV, S_WOB, S_C00, S_C01, S_C10, S_C11 = range(12)

        def kv_issue(gi, ci, slot):
            for d in range(ND):
                for j in range(G):
                    n = gi * G + j
                    rows = pl.ds(ci * R + d * DR, DR)
                    pltpu.make_async_copy(k_hbm.at[n, rows, :], kbuf.at[slot, j, pl.ds(d * DR, DR), :],
                                          kv_sem.at[0, slot]).start(priority=0)
                    pltpu.make_async_copy(v_hbm.at[n, rows, :], vbuf.at[slot, j, pl.ds(d * DR, DR), :],
                                          kv_sem.at[1, slot]).start(priority=1)

        def kv_wait(slot):
            pltpu.make_async_copy(kbuf.at[slot], kbuf.at[slot], kv_sem.at[0, slot]).wait()
            pltpu.make_async_copy(vbuf.at[slot], vbuf.at[slot], kv_sem.at[1, slot]).wait()

        def side_desc(name, idx):
            if name == "wo":
                r = pl.ds(idx * 32, 32)
                return pltpu.make_async_copy(wo_hbm.at[r, :], wo_v.at[r, :], misc_sem.at[S_WO])
            if name == "wob":
                r = pl.ds(idx * 32, 32)
                return pltpu.make_async_copy(wob_hbm.at[r, :], wob_v.at[r, :], misc_sem.at[S_WOB])
            if name in ("wqb", "wuk", "wuv"):
                src, dst, sem = {"wqb": (wqb_hbm, wqb_v, S_WQB), "wuk": (wuk_hbm, wuk_v, S_WUK),
                                 "wuv": (wuv_hbm, wuv_v, S_WUV)}[name]
                r = pl.ds(idx * 128, 128)
                return pltpu.make_async_copy(src.at[r, :], dst.at[r, :], misc_sem.at[sem])
            _, b, hf = name
            r = pl.ds(hf * (SK // 2) + idx * 32, 32)
            return pltpu.make_async_copy(c_hbm.at[b, r, :], c_v.at[b, r, :], misc_sem.at[S_C00 + 2 * b + hf])

        def side_wait(name):
            if name == "wo":
                pltpu.make_async_copy(wo_v, wo_v, misc_sem.at[S_WO]).wait()
            elif name == "wob":
                pltpu.make_async_copy(wob_v, wob_v, misc_sem.at[S_WOB]).wait()
            elif name == "wqb":
                pltpu.make_async_copy(wqb_v, wqb_v, misc_sem.at[S_WQB]).wait()
            elif name == "wuk":
                pltpu.make_async_copy(wuk_v, wuk_v, misc_sem.at[S_WUK]).wait()
            elif name == "wuv":
                pltpu.make_async_copy(wuv_v, wuv_v, misc_sem.at[S_WUV]).wait()
            else:
                _, b, hf = name
                r = pl.ds(hf * (SK // 2), SK // 2)
                pltpu.make_async_copy(c_v.at[b, r, :], c_v.at[b, r, :], misc_sem.at[S_C00 + 2 * b + hf]).wait()

        def side_issue(name, c0):
            for t in range(SPS):
                side_desc(name, c0 * SPS + t).start(priority=t % 2)

        row8 = lax.broadcasted_iota(jnp.int32, (G, DH), 0)
        row8_m = lax.broadcasted_iota(jnp.int32, (G, DM), 0)
        row16_m = lax.broadcasted_iota(jnp.int32, (2 * G, DM), 0)
        row16_d = lax.broadcasted_iota(jnp.int32, (2 * G, DH), 0)

        pltpu.make_async_copy(xa_hbm, xa_v, misc_sem.at[S_XA]).start()
        pltpu.make_async_copy(xb_hbm, xb_v, misc_sem.at[S_XB]).start()
        for t in range(32):
            r = pl.ds(t * 16, 16)
            pltpu.make_async_copy(wq_hbm.at[r, :], wq_v.at[r, :], misc_sem.at[S_WQ]).start(priority=t % 2)
        for i in range(LA):
            kv_issue(i // NC, i % NC, i % NS)

        mb_s[...] = jnp.full(mb_s.shape, -jnp.inf, F32)
        lb_s[...] = jnp.zeros(lb_s.shape, F32)
        accb_s[...] = jnp.zeros(accb_s.shape, F32)
        qb_s[...] = jnp.zeros(qb_s.shape, F32)
        qabs_s[...] = jnp.zeros(qabs_s.shape, F32)
        ctx_s[...] = jnp.zeros(ctx_s.shape, F32)
        outb_s[...] = jnp.zeros(outb_s.shape, F32)

        pltpu.make_async_copy(xa_v, xa_v, misc_sem.at[S_XA]).wait()
        pltpu.make_async_copy(xb_v, xb_v, misc_sem.at[S_XB]).wait()
        pltpu.make_async_copy(wq_v, wq_v, misc_sem.at[S_WQ]).wait()

        def q_group(g):
            b, hg = divmod(g, NH // G)
            xrow = jnp.broadcast_to(xa_v[b:b + 1, :].astype(F32), (G, DM))
            q = jnp.zeros((G, DH), F32)
            for j in range(G):
                h = hg * G + j
                lhs = jnp.where(row8_m == j, xrow, 0.0).astype(BF16)
                q = q + jnp.dot(lhs, wq_v[:, h * DH:(h + 1) * DH], preferred_element_type=F32)
            return q.astype(BF16)

        def pair_weights(w_v, j2):
            u = w_v.bitcast(jnp.uint32)[pl.ds(j2, DM, stride=NH // 2), :]
            ev = pltpu.bitcast(u << 16, F32).astype(BF16)
            od = pltpu.bitcast(u & jnp.uint32(0xFFFF0000), F32).astype(BF16)
            return ev, od

        def b1(j2):
            x0 = jnp.broadcast_to(xb_v[0:1, :].astype(F32), (2 * G, DM))
            x1 = jnp.broadcast_to(xb_v[1:2, :].astype(F32), (2 * G, DM))
            hg = j2 // (G // 2)
            acc = qb_s[hg]
            for e, w in enumerate(pair_weights(wqb_v, j2)):
                jl = (2 * j2 + e) % G
                lhs = jnp.where(row16_m == jl, x0, jnp.where(row16_m == G + jl, x1, 0.0)).astype(BF16)
                acc = acc + jnp.dot(lhs, w, preferred_element_type=F32)
            qb_s[hg] = acc

        def b2(j2):
            hg = j2 // (G // 2)
            qb = qb_s[hg].astype(BF16).astype(F32)
            acc = qabs_s[hg]
            for e, w in enumerate(pair_weights(wuk_v, j2)):
                jl = (2 * j2 + e) % G
                lhs = jnp.where((row16_d == jl) | (row16_d == G + jl), qb, 0.0).astype(BF16)
                acc = acc + lax.dot_general(lhs, w, NT, preferred_element_type=F32)
            qabs_s[hg] = acc

        def b3(b, ch):
            cc = c_v[b, pl.ds(pl.multiple_of(ch * RC, RC), RC), :]
            qa = jnp.concatenate([qabs_s[hg, pl.ds(b * G, G), :] for hg in range(NH // G)], axis=0).astype(BF16)
            s = lax.dot_general(qa, cc, NT, preferred_element_type=F32) * SCALE
            m_prev = mb_s[b]
            m_new = jnp.maximum(m_prev, jnp.max(s, axis=1, keepdims=True))
            alpha = jnp.exp(m_prev - m_new)
            p = jnp.exp(s - m_new)
            lb_s[b] = alpha * lb_s[b] + jnp.sum(p, axis=1, keepdims=True)
            mb_s[b] = m_new
            accb_s[b] = alpha * accb_s[b] + jnp.dot(p.astype(BF16), cc, preferred_element_type=F32)

        def b4(j2):
            hg = j2 // (G // 2)
            r0 = pl.ds(pl.multiple_of(hg * G, G), G)
            cc = jnp.concatenate([accb_s[0, r0, :] / lb_s[0, r0, :], accb_s[1, r0, :] / lb_s[1, r0, :]], axis=0)
            acc = ctx_s[hg]
            for e, w in enumerate(pair_weights(wuv_v, j2)):
                jl = (2 * j2 + e) % G
                lhs = jnp.where((row16_m == jl) | (row16_m == G + jl), cc, 0.0).astype(BF16)
                acc = acc + jnp.dot(lhs, w, preferred_element_type=F32)
            ctx_s[hg] = acc

        def b5(j2):
            hg = j2 // (G // 2)
            ctx = ctx_s[hg].astype(BF16).astype(F32)
            acc = outb_s[...]
            for e in range(2):
                h = 2 * j2 + e
                jl = h % G
                lhs = jnp.where((row16_d == jl) | (row16_d == G + jl), ctx, 0.0).astype(BF16)
                w = wob_v[pl.ds(pl.multiple_of(h * DH, DH), DH), :]
                acc = acc + jnp.dot(lhs, w, preferred_element_type=F32)
            outb_s[...] = acc

        def when_range(c, lo, hi, fn):
            @pl.when((c >= lo) & (c < hi))
            def _():
                fn(c - lo)

        def when_eq(c, v, fn):
            @pl.when(c == v)
            def _():
                fn()

        def sc(x):
            return x * NC // 32

        def extras(g, c):
            if not side_on:
                return
            first = lambda name: when_range(c, 0, HALF, lambda c0: side_issue(name, c0))
            second = lambda name: when_range(c, HALF, NC, lambda c0: side_issue(name, c0))
            W = LA + 1
            def comp(lo, n, fn, static=True):
                if dma_only:
                    return
                stride = max(1, NC // 32)
                if static:
                    for t in range(n):
                        when_eq(c, lo + t * stride, functools.partial(fn, t))
                    return
                @pl.when((c >= lo) & (c < lo + n * stride) & ((c - lo) % stride == 0))
                def _():
                    fn((c - lo) // stride)
            if g == 0:
                first("wo"); second("wqb")
                when_eq(c, NC - 1, lambda: side_wait("wo"))
            elif g == 1:
                first("wuk"); second(("c", 1, 0))
                when_eq(c, W, lambda: side_wait("wqb"))
                comp(sc(4) if sc(4) >= W else W, 16, b1)
            elif g == 2:
                first(("c", 1, 1)); second(("c", 0, 0))
                when_eq(c, 0, lambda: side_wait("wuk"))
                comp(0, 16, b2)
                when_eq(c, sc(16), lambda: side_wait(("c", 1, 0)))
                comp(sc(16), NCH // 2, lambda u: b3(1, u))
            elif g == 3:
                first(("c", 0, 1)); second("wuv")
                when_eq(c, 0, lambda: side_wait(("c", 1, 1)))
                comp(0, NCH // 2, lambda u: b3(1, NCH // 2 + u))
                when_eq(c, sc(8), lambda: side_wait(("c", 0, 0)))
                comp(sc(8), NCH // 2, lambda u: b3(0, u))
            elif g == 4:
                first("wob")
                when_eq(c, 0, lambda: side_wait(("c", 0, 1)))
                comp(0, NCH // 2, lambda u: b3(0, NCH // 2 + u))
                when_eq(c, sc(8), lambda: side_wait("wuv"))
                comp(sc(8), 16, b4)
            elif g == 5:
                when_eq(c, 0, lambda: side_wait("wob"))
                comp(0, 16, b5)

        outa = [jnp.zeros((G, DM), F32) for _ in range(NB)]
        for g in range(NG):
            q = q_group(g) if not dma_only else jnp.zeros((G, DH), BF16)

            def body(c, carry, g=g, q=q):
                m, l, acc = carry
                i = g * NC + c
                slot = i % NS
                nxt = i + LA
                if g == NG - 1:
                    @pl.when(c + LA < NC)
                    def _():
                        kv_issue(nxt // NC, nxt % NC, nxt % NS)
                else:
                    kv_issue(nxt // NC, nxt % NC, nxt % NS)
                extras(g, c)
                kv_wait(slot)
                if dma_only:
                    return m, l, acc + kbuf[slot, 0, 0:G, :].astype(F32) + vbuf[slot, 0, 0:G, :].astype(F32)
                s = None
                rowr = lax.broadcasted_iota(jnp.int32, (G, R), 0)
                for j in range(G):
                    sj = lax.dot_general(q, kbuf[slot, j], NT, preferred_element_type=F32)
                    s = sj if s is None else jnp.where(rowr == j, sj, s)
                s = s * SCALE
                m_new = jnp.maximum(m, jnp.max(s, axis=1, keepdims=True))
                alpha = jnp.exp(m - m_new)
                p = jnp.exp(s - m_new)
                l = alpha * l + jnp.sum(p, axis=1, keepdims=True)
                pb = p.astype(BF16)
                pv = None
                for j in range(G):
                    r = jnp.dot(pb, vbuf[slot, j], preferred_element_type=F32)
                    pv = r if pv is None else jnp.where(row8 == j, r, pv)
                acc = alpha * acc + pv
                return m_new, l, acc

            m0 = jnp.full((G, 1), -jnp.inf, F32)
            l0 = jnp.zeros((G, 1), F32)
            a0 = jnp.zeros((G, DH), F32)
            m, l, acc = lax.fori_loop(0, NC, body, (m0, l0, a0))
            if dma_only:
                outa[0] = outa[0] + jnp.concatenate([acc] * 4, axis=1)
                continue
            b, hg = divmod(g, NH // G)
            o = acc / l
            o = o.astype(BF16).astype(F32)
            for j in range(G):
                h = hg * G + j
                lhs = jnp.where(row8 == j, o, 0.0).astype(BF16)
                outa[b] = outa[b] + jnp.dot(lhs, wo_v[h * DH:(h + 1) * DH, :], preferred_element_type=F32)

        if not side_on:
            pass
        rows = []
        for b in range(NB):
            a = jnp.sum(outa[b], axis=0, keepdims=True)
            bb = jnp.sum(outb_s[pl.ds(b * G, G), :], axis=0, keepdims=True)
            rows.append(jnp.concatenate([a, bb], axis=1))
        out_ref[...] = jnp.concatenate(rows, axis=0).astype(out_ref.dtype)

    any_spec = pl.BlockSpec(memory_space=pl.ANY)
    scratch = [
        pltpu.VMEM((NB, DM), BF16), pltpu.VMEM((NB, DM), BF16),
        pltpu.VMEM((DM, NH * DH), BF16), pltpu.VMEM((NH * DH, DM), BF16),
        pltpu.VMEM((NB, SK, DC), BF16),
        pltpu.VMEM((DM * NH, DH), BF16), pltpu.VMEM((DC * NH, DH), BF16), pltpu.VMEM((DC * NH, DH), BF16),
        pltpu.VMEM((NH * DH, DM), BF16),
        pltpu.VMEM((NS, G, R, DH), BF16), pltpu.VMEM((NS, G, R, DH), BF16),
        pltpu.VMEM((NH // G, 2 * G, DH), F32), pltpu.VMEM((NH // G, 2 * G, DC), F32),
        pltpu.VMEM((NB, NH, 1), F32), pltpu.VMEM((NB, NH, 1), F32), pltpu.VMEM((NB, NH, DC), F32),
        pltpu.VMEM((NH // G, 2 * G, DH), F32), pltpu.VMEM((2 * G, DM), F32),
        pltpu.SemaphoreType.DMA((2, NS)), pltpu.SemaphoreType.DMA((12,)),
    ]

    def run(A_x, A_k_cache, A_v_cache, A_wq, A_wo, B_x, B_c_kv, B_w_q, B_w_uk, B_w_uv, B_w_o):
        return pl.pallas_call(
            kernel,
            in_specs=[any_spec] * 11,
            out_specs=pl.BlockSpec(memory_space=pltpu.VMEM),
            out_shape=jax.ShapeDtypeStruct((NB, 2 * DM), BF16),
            scratch_shapes=scratch,
            compiler_params=pltpu.CompilerParams(vmem_limit_bytes=vmem_mb * 2**20),
        )(A_x.reshape(NB, DM), A_k_cache.reshape(NB * NH, SK, DH), A_v_cache.reshape(NB * NH, SK, DH), A_wq, A_wo,
          B_x.reshape(NB, DM), B_c_kv, B_w_q.reshape(DM * NH, DH), B_w_uk.reshape(DC * NH, DH), B_w_uv.reshape(DC * NH, DH),
          B_w_o.reshape(NH * DH, DM)).reshape(NB, 1, 2 * DM)
    return run


_RUN = build()


@jax.jit
def pallas_concat_heads__gqa_block_cached__compressed_kv_cla__decode_kernel(
    A_x: jax.Array,
    A_k_cache: jax.Array,
    A_v_cache: jax.Array,
    A_wq: jax.Array,
    A_wo: jax.Array,
    B_x: jax.Array,
    B_c_kv: jax.Array,
    B_w_q: jax.Array,
    B_w_uk: jax.Array,
    B_w_uv: jax.Array,
    B_w_o: jax.Array,
):
    return _RUN(A_x, A_k_cache, A_v_cache, A_wq, A_wo, B_x, B_c_kv, B_w_q, B_w_uk, B_w_uv, B_w_o)
```

```python
import functools
import numpy as np
import jax
import jax.numpy as jnp
from jax import lax
from jax.experimental import pallas as pl
from jax.experimental.pallas import tpu as pltpu

F32 = jnp.float32
BF16 = jnp.bfloat16
NT = (((1,), (1,)), ((), ()))

NB, NH, SK, DH = 2, 32, 8192, 128
DM = 512
DC = 512
G = 8
NG = NB * NH // G
HPG = G // NB
SCALE = float(DH) ** -0.5


def build(R=256, DR=128, NS=4, RC=512, vmem_mb=100, dma_only=False, side_inter=True, wq_mode=1, jit_wo=True,
          bounds=True):
    NC = SK // R
    ND = R // DR
    LA = NS - 1
    SIDE = 128
    SPS = SIDE // NC
    NCH = SK // RC
    assert SPS * NC == SIDE

    def kernel(xa_hbm, k_hbm, v_hbm, wq_hbm, wo_hbm, xb_hbm, c_hbm, wqb_hbm, wuk_hbm, wuv_hbm, wob_hbm,
               out_ref,
               xa_v, xb_v, wq_v, wo_v, c_v, wqb_v, wuk_v, wuv_v, wob_v, kbuf, vbuf,
               qb_s, qabs_s, mb_s, lb_s, accb_s, ctx_s, outb_s,
               kv_sem, misc_sem):
        S_XA, S_XB, S_WQ, S_WQB, S_WUK, S_WUV, S_WOB, S_C00, S_C01, S_C10, S_C11 = range(11)
        S_WO = 11

        def head_of(gi, j):
            return (j // HPG) * NH + NG * (j % HPG) + gi

        def kv_descs(gi, ci, slot):
            out = []
            for d in range(ND):
                for j in range(G):
                    n = head_of(gi, j)
                    rows = pl.ds(ci * R + d * DR, DR)
                    out.append((pltpu.make_async_copy(k_hbm.at[n, rows, :], kbuf.at[slot, j, pl.ds(d * DR, DR), :],
                                                      kv_sem.at[0, slot]), 0))
                    out.append((pltpu.make_async_copy(v_hbm.at[n, rows, :], vbuf.at[slot, j, pl.ds(d * DR, DR), :],
                                                      kv_sem.at[1, slot]), 1))
            return out

        def kv_wait(slot):
            pltpu.make_async_copy(kbuf.at[slot], kbuf.at[slot], kv_sem.at[0, slot]).wait()
            pltpu.make_async_copy(vbuf.at[slot], vbuf.at[slot], kv_sem.at[1, slot]).wait()

        def side_desc(name, idx):
            if name == "wob":
                r = pl.ds(idx * 32, 32)
                return pltpu.make_async_copy(wob_hbm.at[r, :], wob_v.at[r, :], misc_sem.at[S_WOB])
            if name in ("wqb", "wuk", "wuv"):
                src, dst, sem = {"wqb": (wqb_hbm, wqb_v, S_WQB), "wuk": (wuk_hbm, wuk_v, S_WUK),
                                 "wuv": (wuv_hbm, wuv_v, S_WUV)}[name]
                r = pl.ds(idx * 128, 128)
                return pltpu.make_async_copy(src.at[r, :], dst.at[r, :], misc_sem.at[sem])
            _, b, hf = name
            r = pl.ds(hf * (SK // 2) + idx * 32, 32)
            return pltpu.make_async_copy(c_hbm.at[b, r, :], c_v.at[b, r, :], misc_sem.at[S_C00 + 2 * b + hf])

        def side_wait(name):
            if name == "wob":
                pltpu.make_async_copy(wob_v, wob_v, misc_sem.at[S_WOB]).wait()
            elif name == "wqb":
                pltpu.make_async_copy(wqb_v, wqb_v, misc_sem.at[S_WQB]).wait()
            elif name == "wuk":
                pltpu.make_async_copy(wuk_v, wuk_v, misc_sem.at[S_WUK]).wait()
            elif name == "wuv":
                pltpu.make_async_copy(wuv_v, wuv_v, misc_sem.at[S_WUV]).wait()
            else:
                _, b, hf = name
                r = pl.ds(hf * (SK // 2), SK // 2)
                pltpu.make_async_copy(c_v.at[b, r, :], c_v.at[b, r, :], misc_sem.at[S_C00 + 2 * b + hf]).wait()

        def wo_descs(g):
            out = []
            for t in range(4):
                for jh in range(HPG):
                    h = g + NG * jh
                    r = pl.ds(h * DH + t * 32, 32)
                    out.append((pltpu.make_async_copy(wo_hbm.at[r, :], wo_v.at[r, :], misc_sem.at[S_WO + g]), jh % 2))
            return out

        def wo_wait(g):
            for jh in range(HPG):
                h = g + NG * jh
                r = pl.ds(h * DH, DH)
                pltpu.make_async_copy(wo_v.at[r, :], wo_v.at[r, :], misc_sem.at[S_WO + g]).wait()

        row8 = lax.broadcasted_iota(jnp.int32, (G, DH), 0)
        row8_m = lax.broadcasted_iota(jnp.int32, (G, DM), 0)
        row16_m = lax.broadcasted_iota(jnp.int32, (2 * G, DM), 0)
        row16_d = lax.broadcasted_iota(jnp.int32, (2 * G, DH), 0)

        pltpu.make_async_copy(xa_hbm, xa_v, misc_sem.at[S_XA]).start()
        pltpu.make_async_copy(xb_hbm, xb_v, misc_sem.at[S_XB]).start()
        if wq_mode == 0:
            for t in range(32):
                r = pl.ds(t * 16, 16)
                pltpu.make_async_copy(wq_hbm.at[r, :], wq_v.at[r, :], misc_sem.at[S_WQ]).start(priority=t % 2)
        elif wq_mode == 1:
            for cb in range(4):
                for t in range(16):
                    tt = (t % 4) * 4 + t // 4
                    for w in range(2):
                        r = pl.ds(w * 256 + tt * 16, 16)
                        cc = pl.ds(cb * 1024, 1024)
                        pltpu.make_async_copy(wq_hbm.at[r, cc], wq_v.at[r, cc], misc_sem.at[S_WQ]).start(priority=w)
        elif wq_mode == 2:
            for t in range(64):
                tt = (t % 8) * 8 + t // 8
                for w in range(2):
                    r = pl.ds(tt * 8, 8)
                    cc = pl.ds(w * 2048, 2048)
                    pltpu.make_async_copy(wq_hbm.at[r, cc], wq_v.at[r, cc], misc_sem.at[S_WQ]).start(priority=w)
        for i in range(LA):
            for cp, pr in kv_descs(i // NC, i % NC, i % NS):
                cp.start(priority=pr)

        mb_s[...] = jnp.full(mb_s.shape, -jnp.inf, F32)
        lb_s[...] = jnp.zeros(lb_s.shape, F32)
        accb_s[...] = jnp.zeros(accb_s.shape, F32)
        qb_s[...] = jnp.zeros(qb_s.shape, F32)
        qabs_s[...] = jnp.zeros(qabs_s.shape, F32)
        ctx_s[...] = jnp.zeros(ctx_s.shape, F32)
        outb_s[...] = jnp.zeros(outb_s.shape, F32)

        pltpu.make_async_copy(xa_hbm, xa_v, misc_sem.at[S_XA]).wait()
        pltpu.make_async_copy(xb_hbm, xb_v, misc_sem.at[S_XB]).wait()
        pltpu.make_async_copy(wq_v, wq_v, misc_sem.at[S_WQ]).wait()

        def q_group(g):
            x0 = jnp.broadcast_to(xa_v[0:1, :].astype(F32), (G, DM))
            x1 = jnp.broadcast_to(xa_v[1:2, :].astype(F32), (G, DM))
            q = jnp.zeros((G, DH), F32)
            for jh in range(HPG):
                h = g + NG * jh
                lhs = jnp.where(row8_m == jh, x0, jnp.where(row8_m == HPG + jh, x1, 0.0)).astype(BF16)
                q = q + jnp.dot(lhs, wq_v[:, h * DH:(h + 1) * DH], preferred_element_type=F32)
            return q.astype(BF16)

        def pair_weights(w_v, j2):
            u = w_v.bitcast(jnp.uint32)[pl.ds(j2, DM, stride=NH // 2), :]
            ev = pltpu.bitcast(u << 16, F32).astype(BF16)
            od = pltpu.bitcast(u & jnp.uint32(0xFFFF0000), F32).astype(BF16)
            return ev, od

        def b1(j2):
            x0 = jnp.broadcast_to(xb_v[0:1, :].astype(F32), (2 * G, DM))
            x1 = jnp.broadcast_to(xb_v[1:2, :].astype(F32), (2 * G, DM))
            hg = j2 // (G // 2)
            acc = qb_s[hg]
            for e, w in enumerate(pair_weights(wqb_v, j2)):
                jl = (2 * j2 + e) % G
                lhs = jnp.where(row16_m == jl, x0, jnp.where(row16_m == G + jl, x1, 0.0)).astype(BF16)
                acc = acc + jnp.dot(lhs, w, preferred_element_type=F32)
            qb_s[hg] = acc

        def b2(j2):
            hg = j2 // (G // 2)
            qb = qb_s[hg].astype(BF16).astype(F32)
            acc = qabs_s[hg]
            for e, w in enumerate(pair_weights(wuk_v, j2)):
                jl = (2 * j2 + e) % G
                lhs = jnp.where((row16_d == jl) | (row16_d == G + jl), qb, 0.0).astype(BF16)
                acc = acc + lax.dot_general(lhs, w, NT, preferred_element_type=F32)
            qabs_s[hg] = acc

        def b3(b, ch):
            cc = c_v[b, pl.ds(pl.multiple_of(ch * RC, RC), RC), :]
            qa = jnp.concatenate([qabs_s[hg, pl.ds(b * G, G), :] for hg in range(NH // G)], axis=0).astype(BF16)
            s = lax.dot_general(qa, cc, NT, preferred_element_type=F32) * SCALE
            m_prev = mb_s[b]
            m_new = jnp.maximum(m_prev, jnp.max(s, axis=1, keepdims=True))
            alpha = jnp.exp(m_prev - m_new)
            p = jnp.exp(s - m_new)
            lb_s[b] = alpha * lb_s[b] + jnp.sum(p, axis=1, keepdims=True)
            mb_s[b] = m_new
            accb_s[b] = alpha * accb_s[b] + jnp.dot(p.astype(BF16), cc, preferred_element_type=F32)

        def b4(j2):
            hg = j2 // (G // 2)
            r0 = pl.ds(hg * G, G)
            cc = jnp.concatenate([accb_s[0, r0, :] / lb_s[0, r0, :], accb_s[1, r0, :] / lb_s[1, r0, :]], axis=0)
            acc = ctx_s[hg]
            for e, w in enumerate(pair_weights(wuv_v, j2)):
                jl = (2 * j2 + e) % G
                lhs = jnp.where((row16_m == jl) | (row16_m == G + jl), cc, 0.0).astype(BF16)
                acc = acc + jnp.dot(lhs, w, preferred_element_type=F32)
            ctx_s[hg] = acc

        def b5(j2):
            hg = j2 // (G // 2)
            ctx = ctx_s[hg].astype(BF16).astype(F32)
            acc = outb_s[...]
            for e in range(2):
                h = 2 * j2 + e
                jl = h % G
                lhs = jnp.where((row16_d == jl) | (row16_d == G + jl), ctx, 0.0).astype(BF16)
                acc = acc + jnp.dot(lhs, wob_v[h * DH:(h + 1) * DH, :], preferred_element_type=F32)
            outb_s[...] = acc

        def when_eq(c, v, fn):
            @pl.when(c == v)
            def _():
                fn()

        side_plan = {0: ("wqb", "wuk"), 1: (("c", 0, 0), ("c", 1, 0)), 2: (("c", 0, 1), ("c", 1, 1)),
                     3: ("wuv", "wob")}
        W = LA + 1

        def extras(g, c):
            def comp(lo, n, fn, static=True):
                if dma_only:
                    return
                if static:
                    for t in range(n):
                        when_eq(c, lo + t, functools.partial(fn, t))
                    return
                @pl.when((c >= lo) & (c < lo + n))
                def _():
                    fn(c - lo)
            if g == 1:
                when_eq(c, W, lambda: side_wait("wqb"))
                comp(W, 16, b1)
            elif g == 2:
                when_eq(c, 0, lambda: side_wait("wuk"))
                comp(0, 16, b2)
                when_eq(c, 16, lambda: (side_wait(("c", 0, 0)), side_wait(("c", 1, 0))))
                comp(16, NCH, lambda u: b3(u % 2, u // 2), static=False)
            elif g == 3:
                when_eq(c, W, lambda: (side_wait(("c", 0, 1)), side_wait(("c", 1, 1))))
                comp(W, NCH, lambda u: b3(u % 2, NCH // 2 + u // 2), static=False)
            elif g == 4:
                when_eq(c, W, lambda: side_wait("wuv"))
                comp(W, 16, b4)
            elif g == 5:
                when_eq(c, 0, lambda: side_wait("wob"))
                comp(0, 16, b5)

        def issue(g, c):
            i = g * NC + c
            nxt = i + LA
            side = []
            if g in side_plan:
                X, Y = side_plan[g]
                for t in range(SPS):
                    side.append((side_desc(X, c + NC * t), 0))
                    side.append((side_desc(Y, c + NC * t), 1))

            def go():
                kv = kv_descs(nxt // NC, nxt % NC, nxt % NS)
                if side and side_inter:
                    npair = len(kv) // 2
                    every = npair // SPS
                    k = 0
                    for t in range(npair):
                        for cp, pr in kv[2 * t:2 * t + 2]:
                            cp.start(priority=pr)
                        if t % every == every - 1:
                            for cp, pr in side[2 * k:2 * k + 2]:
                                cp.start(priority=pr)
                            k += 1
                else:
                    for cp, pr in kv + side:
                        cp.start(priority=pr)
            if g == NG - 1:
                @pl.when(c + LA < NC)
                def _():
                    go()
            else:
                go()
            @pl.when(c == NC - 1 - LA + 0)
            def _():
                if jit_wo:
                    for cp, pr in wo_descs(g):
                        cp.start(priority=pr)

        if not jit_wo:
            for g in range(NG):
                for cp, pr in wo_descs(g):
                    cp.start(priority=pr)

        outa = jnp.zeros((G, DM), F32)
        for g in range(NG):
            q = q_group(g) if not dma_only else jnp.zeros((G, DH), BF16)

            def body(c, carry, g=g, q=q):
                m, l, acc = carry
                slot = (g * NC + c) % NS
                issue(g, c)
                extras(g, c)
                kv_wait(slot)
                if dma_only:
                    return m, l, acc + kbuf[slot, 0, 0:G, :].astype(F32) + vbuf[slot, 0, 0:G, :].astype(F32)
                s = None
                rowr = lax.broadcasted_iota(jnp.int32, (G, R), 0)
                for j in range(G):
                    sj = lax.dot_general(q, kbuf[slot, j], NT, preferred_element_type=F32)
                    s = sj if s is None else jnp.where(rowr == j, sj, s)
                s = s * SCALE
                m_new = jnp.maximum(m, jnp.max(s, axis=1, keepdims=True))
                alpha = jnp.exp(m - m_new)
                p = jnp.exp(s - m_new)
                l = alpha * l + jnp.sum(p, axis=1, keepdims=True)
                pb = p.astype(BF16)
                pv = None
                for j in range(G):
                    r = jnp.dot(pb, vbuf[slot, j], preferred_element_type=F32)
                    pv = r if pv is None else jnp.where(row8 == j, r, pv)
                acc = alpha * acc + pv
                return m_new, l, acc

            m0 = jnp.full((G, 1), -jnp.inf, F32)
            l0 = jnp.zeros((G, 1), F32)
            a0 = jnp.zeros((G, DH), F32)
            m, l, acc = lax.fori_loop(0, NC, body, (m0, l0, a0))
            wo_wait(g)
            if dma_only:
                outa = outa + jnp.concatenate([acc] * 4, axis=1)
                continue
            o = (acc / l).astype(BF16).astype(F32)
            for jh in range(HPG):
                h = g + NG * jh
                lhs = jnp.where((row8 == jh) | (row8 == HPG + jh), o, 0.0).astype(BF16)
                outa = outa + jnp.dot(lhs, wo_v[h * DH:(h + 1) * DH, :], preferred_element_type=F32)

        rows = []
        for b in range(NB):
            a = jnp.sum(jnp.where(row8_m // HPG == b, outa, 0.0), axis=0, keepdims=True)
            bb = jnp.sum(outb_s[pl.ds(b * G, G), :], axis=0, keepdims=True)
            rows.append(jnp.concatenate([a, bb], axis=1))
        out_ref[...] = jnp.concatenate(rows, axis=0).astype(out_ref.dtype)

    any_spec = pl.BlockSpec(memory_space=pl.ANY)
    scratch = [
        pltpu.VMEM((NB, DM), BF16), pltpu.VMEM((NB, DM), BF16),
        pltpu.VMEM((DM, NH * DH), BF16), pltpu.VMEM((NH * DH, DM), BF16),
        pltpu.VMEM((NB, SK, DC), BF16),
        pltpu.VMEM((DM * NH, DH), BF16), pltpu.VMEM((DC * NH, DH), BF16), pltpu.VMEM((DC * NH, DH), BF16),
        pltpu.VMEM((NH * DH, DM), BF16),
        pltpu.VMEM((NS, G, R, DH), BF16), pltpu.VMEM((NS, G, R, DH), BF16),
        pltpu.VMEM((NH // G, 2 * G, DH), F32), pltpu.VMEM((NH // G, 2 * G, DC), F32),
        pltpu.VMEM((NB, NH, 1), F32), pltpu.VMEM((NB, NH, 1), F32), pltpu.VMEM((NB, NH, DC), F32),
        pltpu.VMEM((NH // G, 2 * G, DH), F32), pltpu.VMEM((2 * G, DM), F32),
        pltpu.SemaphoreType.DMA((2, NS)), pltpu.SemaphoreType.DMA((11 + NG,)),
    ]

    def run(A_x, A_k_cache, A_v_cache, A_wq, A_wo, B_x, B_c_kv, B_w_q, B_w_uk, B_w_uv, B_w_o):
        return pl.pallas_call(
            kernel,
            in_specs=[any_spec] * 11,
            out_specs=pl.BlockSpec(memory_space=pltpu.VMEM),
            out_shape=jax.ShapeDtypeStruct((NB, 2 * DM), BF16),
            scratch_shapes=scratch,
            compiler_params=pltpu.CompilerParams(vmem_limit_bytes=vmem_mb * 2**20, disable_bounds_checks=not bounds),
        )(A_x.reshape(NB, DM), A_k_cache.reshape(NB * NH, SK, DH), A_v_cache.reshape(NB * NH, SK, DH), A_wq, A_wo,
          B_x.reshape(NB, DM), B_c_kv, B_w_q.reshape(DM * NH, DH), B_w_uk.reshape(DC * NH, DH),
          B_w_uv.reshape(DC * NH, DH), B_w_o.reshape(NH * DH, DM)).reshape(NB, 1, 2 * DM)
    return run


_RUN = build(wq_mode=0)


@jax.jit
def pallas_concat_heads__gqa_block_cached__compressed_kv_cla__decode_kernel(
    A_x: jax.Array,
    A_k_cache: jax.Array,
    A_v_cache: jax.Array,
    A_wq: jax.Array,
    A_wo: jax.Array,
    B_x: jax.Array,
    B_c_kv: jax.Array,
    B_w_q: jax.Array,
    B_w_uk: jax.Array,
    B_w_uv: jax.Array,
    B_w_o: jax.Array,
):
    return _RUN(A_x, A_k_cache, A_v_cache, A_wq, A_wo, B_x, B_c_kv, B_w_q, B_w_uk, B_w_uv, B_w_o)
```

```python
import functools

import jax
import jax.numpy as jnp
from jax import lax
from jax.experimental import pallas as pl
from jax.experimental.pallas import tpu as pltpu

F32 = jnp.float32
BF16 = jnp.bfloat16
NT = (((1,), (1,)), ((), ()))

NB, NH, SK, DH = 2, 32, 8192, 128
DM = 512
DC = 512
G = 8
NG = NB * NH // G
HPG = G // NB
SCALE = float(DH) ** -0.5


def build(R=256, DR=128, NS=4, RC=512, vmem_mb=100, dma_only=False, wq_step=8, RL=64, HP=4, scopes=False, s_wl=1, s_hp=1, s_at=2):
    NC = SK // R
    ND = R // DR
    LA = NS - 1
    SIDE = 128
    SPS = SIDE // NC
    NCH = SK // RC
    assert SPS * NC == SIDE and NC == 32 and LA < NC

    def kernel(xa_hbm, k_hbm, v_hbm, wq_hbm, wo_hbm, xb_hbm, c_hbm, wqb_hbm, wuk_hbm, wuv_hbm, wob_hbm,
               out_ref,
               xa_v, xb_v, wq_v, wo_v, c_v, wqb_v, wuk_v, wuv_v, wob_v, kbuf, vbuf,
               wt_s, qb_s, qabs_s, mb_s, lb_s, accb_s, ctx_s, outb_s,
               kv_sem, misc_sem):
        S_XA, S_XB, S_WQB, S_WUK, S_WUV, S_WOB, S_C = range(7)
        S_WO = S_C + 4
        S_WQ = S_WO + NG

        def kv_descs(gi, ci, slot):
            out = []
            for d in range(ND):
                for j in range(G):
                    b, h = j // HPG, gi + NG * (j % HPG)
                    rows = pl.ds(ci * R + d * DR, DR)
                    dst = pl.ds(d * DR, DR)
                    out.append((pltpu.make_async_copy(k_hbm.at[b, h, rows, :], kbuf.at[slot, j, dst, :],
                                                      kv_sem.at[0, slot]), 0))
                    out.append((pltpu.make_async_copy(v_hbm.at[b, h, rows, :], vbuf.at[slot, j, dst, :],
                                                      kv_sem.at[1, slot]), 1))
            return out

        def kv_wait(slot):
            pltpu.make_async_copy(kbuf.at[slot], kbuf.at[slot], kv_sem.at[0, slot]).wait()
            pltpu.make_async_copy(vbuf.at[slot], vbuf.at[slot], kv_sem.at[1, slot]).wait()

        head3 = {"wqb": (wqb_hbm, wqb_v, S_WQB), "wuk": (wuk_hbm, wuk_v, S_WUK), "wuv": (wuv_hbm, wuv_v, S_WUV)}

        def side_desc(name, idx):
            if name == "wob":
                h, t = idx // 4, idx % 4
                r = pl.ds(pl.multiple_of(t * 32, 32), 32)
                return pltpu.make_async_copy(wob_hbm.at[h, r, :], wob_v.at[h, r, :], misc_sem.at[S_WOB])
            if name in head3:
                src, dst, sem = head3[name]
                r = pl.ds(idx * 4, 4)
                return pltpu.make_async_copy(src.at[r], dst.at[r], misc_sem.at[sem])
            _, b, hf = name
            r = pl.ds(hf * (SK // 2) + idx * 32, 32)
            return pltpu.make_async_copy(c_hbm.at[b, r, :], c_v.at[b, r, :], misc_sem.at[S_C + 2 * b + hf])

        def side_wait(name):
            if name == "wob":
                buf, sem = wob_v, S_WOB
            elif name in head3:
                buf, sem = head3[name][1], head3[name][2]
            else:
                _, b, hf = name
                buf, sem = c_v.at[b, pl.ds(hf * (SK // 2), SK // 2), :], S_C + 2 * b + hf
            pltpu.make_async_copy(buf, buf, misc_sem.at[sem]).wait()

        def wq_descs(g):
            out = []
            for t in range(4):
                for jh in range(HPG):
                    r, cc = pl.ds(t * 128, 128), pl.ds((g + NG * jh) * DH, DH)
                    out.append((pltpu.make_async_copy(wq_hbm.at[r, cc], wq_v.at[r, cc], misc_sem.at[S_WQ + g]),
                                jh % 2))
            return out

        def wo_descs(g):
            out = []
            for t in range(4):
                for jh in range(HPG):
                    r = pl.ds((g + NG * jh) * DH + t * 32, 32)
                    out.append((pltpu.make_async_copy(wo_hbm.at[r, :], wo_v.at[r, :], misc_sem.at[S_WO + g]),
                                jh % 2))
            return out

        def start_all(descs):
            for cp, prio in descs:
                cp.start(priority=prio)

        def wait_all(descs):
            for cp, _ in descs:
                cp.wait()

        row8 = lax.broadcasted_iota(jnp.int32, (G, DH), 0)
        row8_m = lax.broadcasted_iota(jnp.int32, (G, DM), 0)
        row8_r = lax.broadcasted_iota(jnp.int32, (G, R), 0)
        row16_m = lax.broadcasted_iota(jnp.int32, (2 * G, DM), 0)
        row16_d = lax.broadcasted_iota(jnp.int32, (2 * G, DH), 0)

        x_copies = [pltpu.make_async_copy(xa_hbm, xa_v, misc_sem.at[S_XA]),
                    pltpu.make_async_copy(xb_hbm, xb_v, misc_sem.at[S_XB])]
        for cp in x_copies:
            cp.start()
        start_all(wq_descs(0))

        def first_steps(i, carry):
            start_all(kv_descs(0, i, i))
            return carry
        lax.fori_loop(0, LA, first_steps, 0)

        mb_s[...] = jnp.full(mb_s.shape, -jnp.inf, F32)
        lb_s[...] = jnp.zeros(lb_s.shape, F32)
        accb_s[...] = jnp.zeros(accb_s.shape, F32)
        qb_s[...] = jnp.zeros(qb_s.shape, F32)
        qabs_s[...] = jnp.zeros(qabs_s.shape, F32)
        ctx_s[...] = jnp.zeros(ctx_s.shape, F32)
        outb_s[...] = jnp.zeros(outb_s.shape, F32)
        for cp in x_copies:
            cp.wait()

        def q_group(g):
            x0 = jnp.broadcast_to(xa_v[0:1, :].astype(F32), (G, DM))
            x1 = jnp.broadcast_to(xa_v[1:2, :].astype(F32), (G, DM))
            q = jnp.zeros((G, DH), F32)
            for jh in range(HPG):
                h = g + NG * jh
                lhs = jnp.where(row8_m == jh, x0, jnp.where(row8_m == HPG + jh, x1, 0.0)).astype(BF16)
                q = q + jnp.dot(lhs, wq_v[:, h * DH:(h + 1) * DH], preferred_element_type=F32)
            return q.astype(BF16)

        def keep_rows(rows, jl, x):
            return jnp.where((rows == jl) | (rows == G + jl), x, 0.0).astype(BF16)

        def head_major(w_v, t):
            r = pl.ds(pl.multiple_of(t * RL, RL), RL)
            wt_s[:, r, :] = jnp.swapaxes(w_v[r, :, :], 0, 1)

        def b_query(t):
            x0 = jnp.broadcast_to(xb_v[0:1, :].astype(F32), (2 * G, DM))
            x1 = jnp.broadcast_to(xb_v[1:2, :].astype(F32), (2 * G, DM))
            x01 = jnp.where(row16_m < G, x0, x1)
            hg = HP * t // G
            acc = qb_s[hg]
            for e in range(HP):
                h = HP * t + e
                acc = acc + jnp.dot(keep_rows(row16_m, h % G, x01), wt_s[h], preferred_element_type=F32)
            qb_s[hg] = acc

        def b_absorb(t):
            hg = HP * t // G
            qb = qb_s[hg].astype(BF16).astype(F32)
            acc = qabs_s[hg]
            for e in range(HP):
                h = HP * t + e
                acc = acc + lax.dot_general(keep_rows(row16_d, h % G, qb), wt_s[h], NT, preferred_element_type=F32)
            qabs_s[hg] = acc

        def b_attend(b, ch):
            cc = c_v[b, pl.ds(pl.multiple_of(ch * RC, RC), RC), :]
            qa = jnp.concatenate([qabs_s[hg, pl.ds(pl.multiple_of(b * G, G), G), :] for hg in range(NH // G)],
                                 axis=0).astype(BF16)
            s = lax.dot_general(qa, cc, NT, preferred_element_type=F32) * SCALE
            m_prev = mb_s[b]
            m_new = jnp.maximum(m_prev, jnp.max(s, axis=1, keepdims=True))
            alpha = jnp.exp(m_prev - m_new)
            p = jnp.exp(s - m_new)
            lb_s[b] = alpha * lb_s[b] + jnp.sum(p, axis=1, keepdims=True)
            mb_s[b] = m_new
            accb_s[b] = alpha * accb_s[b] + jnp.dot(p.astype(BF16), cc, preferred_element_type=F32)

        def b_context(t):
            hg = HP * t // G
            r0 = pl.ds(pl.multiple_of(hg * G, G), G)
            cc = jnp.concatenate([accb_s[b, r0, :] / lb_s[b, r0, :] for b in range(NB)], axis=0)
            acc = ctx_s[hg]
            for e in range(HP):
                h = HP * t + e
                acc = acc + jnp.dot(keep_rows(row16_m, h % G, cc), wt_s[h], preferred_element_type=F32)
            ctx_s[hg] = acc

        def b_project(t):
            hg = HP * t // G
            ctx = ctx_s[hg].astype(BF16).astype(F32)
            acc = outb_s[...]
            for e in range(HP):
                h = HP * t + e
                acc = acc + jnp.dot(keep_rows(row16_d, h % G, ctx), wob_v[h], preferred_element_type=F32)
            outb_s[...] = acc

        def at_step(c, v, fn):
            pl.when(c == v)(fn)

        W = LA + 1
        side_plan = {0: ("wqb", "wuk"), 1: (("c", 0, 0), ("c", 1, 0)), 2: (("c", 0, 1), ("c", 1, 1)),
                     3: ("wuv", "wob")}

        half = NB * NCH // 2
        phases = [(NC + W, DM // RL, s_wl, ["wqb"], functools.partial(head_major, wqb_v)),
                  (0, NH // HP, s_hp, [], b_query),
                  (0, DC // RL, s_wl, ["wuk"], functools.partial(head_major, wuk_v)),
                  (0, NH // HP, s_hp, [], b_absorb),
                  (2 * NC + W, half, s_at, [("c", b, 0) for b in range(NB)], lambda u: b_attend(u % NB, u // NB)),
                  (3 * NC + W, half, s_at, [("c", b, 1) for b in range(NB)],
                   lambda u: b_attend(u % NB, NCH // 2 + u // NB)),
                  (4 * NC + W, DC // RL, s_wl, ["wuv"], functools.partial(head_major, wuv_v)),
                  (0, NH // HP, s_hp, [], b_context),
                  (0, NH // HP, s_hp, ["wob"], b_project)]
        plan, nxt_i = [], 0
        for lo, n, stride, names, fn in phases:
            lo = max(lo, nxt_i)
            plan.append((lo, stride, lo + n * stride, names, fn))
            nxt_i = lo + n * stride
        assert nxt_i <= NG * NC

        def b_work(g, c):
            for lo, stride, hi, names, fn in plan:
                if names and lo // NC == g:
                    at_step(c, lo % NC, lambda names=names: [side_wait(n) for n in names] and None)
                a, z = max(lo, g * NC), min(hi, (g + 1) * NC)
                if a < z and not dma_only:
                    i = c + (g * NC - lo)
                    cond = (c >= a - g * NC) & (c < z - g * NC)
                    if stride > 1:
                        cond = cond & (i % stride == 0)
                    pl.when(cond)(functools.partial(fn, i // stride))

        def issue(g, c):
            nxt = g * NC + c + LA

            def go():
                kv = kv_descs(nxt // NC, nxt % NC, nxt % NS)
                if g in side_plan:
                    every = len(kv) // (2 * SPS)
                    for t in range(SPS):
                        start_all(kv[2 * every * t:2 * every * (t + 1)])
                        for prio, name in enumerate(side_plan[g]):
                            side_desc(name, c + NC * t).start(priority=prio)
                else:
                    start_all(kv)
            if g == NG - 1:
                pl.when(c + LA < NC)(go)
            else:
                go()
            if g + 1 < NG:
                at_step(c, wq_step, lambda: start_all(wq_descs(g + 1)))
            at_step(c, NC - 1 - LA, lambda: start_all(wo_descs(g)))

        outa = jnp.zeros((G, DM), F32)
        for g in range(NG):
            wait_all(wq_descs(g))
            q = q_group(g) if not dma_only else jnp.zeros((G, DH), BF16)

            def step(c, carry, g=g, q=q):
                m, l, acc = carry
                slot = (g * NC + c) % NS
                issue(g, c)
                b_work(g, c)
                kv_wait(slot)
                if dma_only:
                    return m, l, acc + kbuf[slot, 0, 0:G, :].astype(F32) + vbuf[slot, 0, 0:G, :].astype(F32)
                s = None
                for j in range(G):
                    sj = lax.dot_general(q, kbuf[slot, j], NT, preferred_element_type=F32)
                    s = sj if s is None else jnp.where(row8_r == j, sj, s)
                s = s * SCALE
                m_new = jnp.maximum(m, jnp.max(s, axis=1, keepdims=True))
                alpha = jnp.exp(m - m_new)
                p = jnp.exp(s - m_new)
                l = alpha * l + jnp.sum(p, axis=1, keepdims=True)
                pb = p.astype(BF16)
                pv = None
                for j in range(G):
                    r = jnp.dot(pb, vbuf[slot, j], preferred_element_type=F32)
                    pv = r if pv is None else jnp.where(row8 == j, r, pv)
                return m_new, l, alpha * acc + pv

            init = (jnp.full((G, 1), -jnp.inf, F32), jnp.zeros((G, 1), F32), jnp.zeros((G, DH), F32))
            if scopes:
                with jax.named_scope("loop%d" % g):
                    m, l, acc = lax.fori_loop(0, NC, step, init)
            else:
                m, l, acc = lax.fori_loop(0, NC, step, init)
            wait_all(wo_descs(g))
            if dma_only:
                outa = outa + jnp.concatenate([acc] * 4, axis=1)
                continue
            o = (acc / l).astype(BF16).astype(F32)
            for jh in range(HPG):
                h = g + NG * jh
                lhs = jnp.where((row8 == jh) | (row8 == HPG + jh), o, 0.0).astype(BF16)
                outa = outa + jnp.dot(lhs, wo_v[h * DH:(h + 1) * DH, :], preferred_element_type=F32)

        rows = []
        for b in range(NB):
            a = jnp.sum(jnp.where(row8_m // HPG == b, outa, 0.0), axis=0, keepdims=True)
            bb = jnp.sum(outb_s[pl.ds(b * G, G), :], axis=0, keepdims=True)
            rows.append(jnp.concatenate([a, bb], axis=1))
        out_ref[...] = jnp.concatenate(rows, axis=0).astype(out_ref.dtype)

    scratch = [
        pltpu.VMEM((NB, DM), BF16), pltpu.VMEM((NB, DM), BF16),
        pltpu.VMEM((DM, NH * DH), BF16), pltpu.VMEM((NH * DH, DM), BF16),
        pltpu.VMEM((NB, SK, DC), BF16),
        pltpu.VMEM((DM, NH, DH), BF16), pltpu.VMEM((DC, NH, DH), BF16), pltpu.VMEM((DC, NH, DH), BF16),
        pltpu.VMEM((NH, DH, DM), BF16),
        pltpu.VMEM((NS, G, R, DH), BF16), pltpu.VMEM((NS, G, R, DH), BF16),
        pltpu.VMEM((NH, DM, DH), BF16),
        pltpu.VMEM((NH // G, 2 * G, DH), F32), pltpu.VMEM((NH // G, 2 * G, DC), F32),
        pltpu.VMEM((NB, NH, 1), F32), pltpu.VMEM((NB, NH, 1), F32), pltpu.VMEM((NB, NH, DC), F32),
        pltpu.VMEM((NH // G, 2 * G, DH), F32), pltpu.VMEM((2 * G, DM), F32),
        pltpu.SemaphoreType.DMA((2, NS)), pltpu.SemaphoreType.DMA((10 + 2 * NG,)),
    ]

    def run(A_x, A_k_cache, A_v_cache, A_wq, A_wo, B_x, B_c_kv, B_w_q, B_w_uk, B_w_uv, B_w_o):
        out = pl.pallas_call(
            kernel,
            in_specs=[pl.BlockSpec(memory_space=pl.ANY)] * 11,
            out_specs=pl.BlockSpec(memory_space=pltpu.VMEM),
            out_shape=jax.ShapeDtypeStruct((NB, 2 * DM), BF16),
            scratch_shapes=scratch,
            compiler_params=pltpu.CompilerParams(vmem_limit_bytes=vmem_mb * 2**20),
        )(A_x.reshape(NB, DM), A_k_cache, A_v_cache, A_wq, A_wo,
          B_x.reshape(NB, DM), B_c_kv, B_w_q, B_w_uk, B_w_uv, B_w_o)
        return out.reshape(NB, 1, 2 * DM)
    return run


_RUN = build()


@jax.jit
def pallas_concat_heads__gqa_block_cached__compressed_kv_cla__decode_kernel(
    A_x: jax.Array,
    A_k_cache: jax.Array,
    A_v_cache: jax.Array,
    A_wq: jax.Array,
    A_wo: jax.Array,
    B_x: jax.Array,
    B_c_kv: jax.Array,
    B_w_q: jax.Array,
    B_w_uk: jax.Array,
    B_w_uv: jax.Array,
    B_w_o: jax.Array,
):
    return _RUN(A_x, A_k_cache, A_v_cache, A_wq, A_wo, B_x, B_c_kv, B_w_q, B_w_uk, B_w_uv, B_w_o)
```

```python
import functools

import jax
import jax.numpy as jnp
from jax import lax
from jax.experimental import pallas as pl
from jax.experimental.pallas import tpu as pltpu

F32 = jnp.float32
BF16 = jnp.bfloat16
NT = (((1,), (1,)), ((), ()))

NB, NH, SK, DH = 2, 32, 8192, 128
DM = 512
DC = 512
G = 8
NG = NB * NH // G
HPG = G // NB
SCALE = float(DH) ** -0.5


def build(R=256, DR=128, NS=4, RC=512, vmem_mb=100, dma_only=False, wq_step=8, RL=64, HP=4, scopes=False, s_wl=1, s_hp=1, s_at=2, nosem=False, nobounds=False, NW=1):
    NC = SK // R
    ND = R // DR
    LA = NS - 1
    SIDE = 128
    SPS = SIDE // NC
    NCH = SK // RC
    assert SPS * NC == SIDE and NC == 32 and LA < NC

    def kernel(xa_hbm, k_hbm, v_hbm, wq_hbm, wo_hbm, xb_hbm, c_hbm, wqb_hbm, wuk_hbm, wuv_hbm, wob_hbm,
               out_ref,
               xa_v, xb_v, wq_v, wo_v, c_v, wqb_v, wuk_v, wuv_v, wob_v, kvbuf,
               wt_s, qb_s, qabs_s, mb_s, lb_s, accb_s, ctx_s, outb_s,
               kv_sem, misc_sem):
        S_W, S_SIDE = 0, NW
        S_WQ = S_W
        S_WO = S_W + NW - 1
        side_plan = {0: ("wqb", "wuk"), 1: (("c", 0, 0), ("c", 1, 0)), 2: (("c", 0, 1), ("c", 1, 1)),
                     3: ("wuv", "wob")}
        side_sem = {name: S_SIDE + 2 * (g % 2) + w for g, names in side_plan.items() for w, name in enumerate(names)}

        def kv_descs(gi, ci, slot):
            out = []
            for d in range(ND):
                for j in range(G):
                    b, h = j // HPG, gi + NG * (j % HPG)
                    rows = pl.ds(ci * R + d * DR, DR)
                    dst = pl.ds(d * DR, DR)
                    for w, src in enumerate((k_hbm, v_hbm)):
                        out.append((pltpu.make_async_copy(src.at[b, h, rows, :], kvbuf.at[slot, w, j, dst, :],
                                                          kv_sem.at[slot]), w))
            return out

        def kv_wait(slot):
            pltpu.make_async_copy(kvbuf.at[slot], kvbuf.at[slot], kv_sem.at[slot]).wait()

        head3 = {"wqb": (wqb_hbm, wqb_v), "wuk": (wuk_hbm, wuk_v), "wuv": (wuv_hbm, wuv_v)}

        def side_desc(name, idx):
            if name == "wob":
                h, t = idx // 4, idx % 4
                r = pl.ds(pl.multiple_of(t * 32, 32), 32)
                src, dst = wob_hbm.at[h, r, :], wob_v.at[h, r, :]
            elif name in head3:
                r = pl.ds(idx * 4, 4)
                src, dst = head3[name][0].at[r], head3[name][1].at[r]
            else:
                _, b, hf = name
                r = pl.ds(hf * (SK // 2) + idx * 32, 32)
                src, dst = c_hbm.at[b, r, :], c_v.at[b, r, :]
            return pltpu.make_async_copy(src, dst, misc_sem.at[side_sem[name]])

        def side_wait(name):
            if name == "wob":
                buf = wob_v
            elif name in head3:
                buf = head3[name][1]
            else:
                _, b, hf = name
                buf = c_v.at[b, pl.ds(hf * (SK // 2), SK // 2), :]
            pltpu.make_async_copy(buf, buf, misc_sem.at[side_sem[name]]).wait()

        def wq_descs(g):
            out = []
            for t in range(4):
                for jh in range(HPG):
                    r, cc = pl.ds(t * 128, 128), pl.ds((g + NG * jh) * DH, DH)
                    out.append((pltpu.make_async_copy(wq_hbm.at[r, cc], wq_v.at[r, cc], misc_sem.at[S_WQ]),
                                jh % 2))
            return out

        def wo_descs(g):
            out = []
            for t in range(4):
                for jh in range(HPG):
                    r = pl.ds((g + NG * jh) * DH + t * 32, 32)
                    out.append((pltpu.make_async_copy(wo_hbm.at[r, :], wo_v.at[r, :], misc_sem.at[S_WO]),
                                jh % 2))
            return out

        def start_all(descs):
            for cp, prio in descs:
                cp.start(priority=prio)

        def wait_all(descs):
            for cp, _ in descs:
                cp.wait()

        row8 = lax.broadcasted_iota(jnp.int32, (G, DH), 0)
        row8_m = lax.broadcasted_iota(jnp.int32, (G, DM), 0)
        row8_r = lax.broadcasted_iota(jnp.int32, (G, R), 0)
        row16_m = lax.broadcasted_iota(jnp.int32, (2 * G, DM), 0)
        row16_d = lax.broadcasted_iota(jnp.int32, (2 * G, DH), 0)

        x_copies = [pltpu.make_async_copy(xa_hbm, xa_v, misc_sem.at[S_W]),
                    pltpu.make_async_copy(xb_hbm, xb_v, misc_sem.at[S_W])]
        for cp in x_copies:
            cp.start()
        start_all(wq_descs(0))

        def first_steps(i, carry):
            start_all(kv_descs(0, i, i))
            return carry
        lax.fori_loop(0, LA, first_steps, 0)

        mb_s[...] = jnp.full(mb_s.shape, -jnp.inf, F32)
        lb_s[...] = jnp.zeros(lb_s.shape, F32)
        accb_s[...] = jnp.zeros(accb_s.shape, F32)
        qb_s[...] = jnp.zeros(qb_s.shape, F32)
        qabs_s[...] = jnp.zeros(qabs_s.shape, F32)
        ctx_s[...] = jnp.zeros(ctx_s.shape, F32)
        outb_s[...] = jnp.zeros(outb_s.shape, F32)
        for cp in x_copies:
            cp.wait()

        def q_group(g):
            x0 = jnp.broadcast_to(xa_v[0:1, :].astype(F32), (G, DM))
            x1 = jnp.broadcast_to(xa_v[1:2, :].astype(F32), (G, DM))
            q = jnp.zeros((G, DH), F32)
            for jh in range(HPG):
                h = g + NG * jh
                lhs = jnp.where(row8_m == jh, x0, jnp.where(row8_m == HPG + jh, x1, 0.0)).astype(BF16)
                q = q + jnp.dot(lhs, wq_v[:, h * DH:(h + 1) * DH], preferred_element_type=F32)
            return q.astype(BF16)

        def keep_rows(rows, jl, x):
            return jnp.where((rows == jl) | (rows == G + jl), x, 0.0).astype(BF16)

        def head_major(w_v, t):
            r = pl.ds(pl.multiple_of(t * RL, RL), RL)
            wt_s[:, r, :] = jnp.swapaxes(w_v[r, :, :], 0, 1)

        def b_query(t):
            x0 = jnp.broadcast_to(xb_v[0:1, :].astype(F32), (2 * G, DM))
            x1 = jnp.broadcast_to(xb_v[1:2, :].astype(F32), (2 * G, DM))
            x01 = jnp.where(row16_m < G, x0, x1)
            hg = HP * t // G
            acc = qb_s[hg]
            for e in range(HP):
                h = HP * t + e
                acc = acc + jnp.dot(keep_rows(row16_m, h % G, x01), wt_s[h], preferred_element_type=F32)
            qb_s[hg] = acc

        def b_absorb(t):
            hg = HP * t // G
            qb = qb_s[hg].astype(BF16).astype(F32)
            acc = qabs_s[hg]
            for e in range(HP):
                h = HP * t + e
                acc = acc + lax.dot_general(keep_rows(row16_d, h % G, qb), wt_s[h], NT, preferred_element_type=F32)
            qabs_s[hg] = acc

        def b_attend(b, ch):
            cc = c_v[b, pl.ds(pl.multiple_of(ch * RC, RC), RC), :]
            qa = jnp.concatenate([qabs_s[hg, pl.ds(pl.multiple_of(b * G, G), G), :] for hg in range(NH // G)],
                                 axis=0).astype(BF16)
            s = lax.dot_general(qa, cc, NT, preferred_element_type=F32) * SCALE
            m_prev = mb_s[b]
            m_new = jnp.maximum(m_prev, jnp.max(s, axis=1, keepdims=True))
            alpha = jnp.exp(m_prev - m_new)
            p = jnp.exp(s - m_new)
            lb_s[b] = alpha * lb_s[b] + jnp.sum(p, axis=1, keepdims=True)
            mb_s[b] = m_new
            accb_s[b] = alpha * accb_s[b] + jnp.dot(p.astype(BF16), cc, preferred_element_type=F32)

        def b_context(t):
            hg = HP * t // G
            r0 = pl.ds(pl.multiple_of(hg * G, G), G)
            cc = jnp.concatenate([accb_s[b, r0, :] / lb_s[b, r0, :] for b in range(NB)], axis=0)
            acc = ctx_s[hg]
            for e in range(HP):
                h = HP * t + e
                acc = acc + jnp.dot(keep_rows(row16_m, h % G, cc), wt_s[h], preferred_element_type=F32)
            ctx_s[hg] = acc

        def b_project(t):
            hg = HP * t // G
            ctx = ctx_s[hg].astype(BF16).astype(F32)
            acc = outb_s[...]
            for e in range(HP):
                h = HP * t + e
                acc = acc + jnp.dot(keep_rows(row16_d, h % G, ctx), wob_v[h], preferred_element_type=F32)
            outb_s[...] = acc

        def at_step(c, v, fn):
            pl.when(c == v)(fn)

        W = LA + 1

        half = NB * NCH // 2
        phases = [(NC + W, DM // RL, s_wl, ["wqb"], functools.partial(head_major, wqb_v)),
                  (0, NH // HP, s_hp, [], b_query),
                  (0, DC // RL, s_wl, ["wuk"], functools.partial(head_major, wuk_v)),
                  (0, NH // HP, s_hp, [], b_absorb),
                  (2 * NC + W, half, s_at, [("c", b, 0) for b in range(NB)], lambda u: b_attend(u % NB, u // NB)),
                  (3 * NC + W, half, s_at, [("c", b, 1) for b in range(NB)],
                   lambda u: b_attend(u % NB, NCH // 2 + u // NB)),
                  (4 * NC + W, DC // RL, s_wl, ["wuv"], functools.partial(head_major, wuv_v)),
                  (0, NH // HP, s_hp, [], b_context),
                  (0, NH // HP, s_hp, ["wob"], b_project)]
        plan, nxt_i = [], 0
        for lo, n, stride, names, fn in phases:
            lo = max(lo, nxt_i)
            plan.append((lo, stride, lo + n * stride, names, fn))
            nxt_i = lo + n * stride
        assert nxt_i <= NG * NC

        def b_work(g, c):
            for lo, stride, hi, names, fn in plan:
                if names and lo // NC == g:
                    at_step(c, lo % NC, lambda names=names: [side_wait(n) for n in names] and None)
                a, z = max(lo, g * NC), min(hi, (g + 1) * NC)
                if a < z and not dma_only:
                    i = c + (g * NC - lo)
                    cond = (c >= a - g * NC) & (c < z - g * NC)
                    if stride > 1:
                        cond = cond & (i % stride == 0)
                    pl.when(cond)(functools.partial(fn, i // stride))

        def issue(g, c):
            nxt = g * NC + c + LA

            def go():
                kv = kv_descs(nxt // NC, nxt % NC, nxt % NS)
                if g in side_plan:
                    every = len(kv) // (2 * SPS)
                    for t in range(SPS):
                        start_all(kv[2 * every * t:2 * every * (t + 1)])
                        for prio, name in enumerate(side_plan[g]):
                            side_desc(name, c + NC * t).start(priority=prio)
                else:
                    start_all(kv)
            if g == NG - 1:
                pl.when(c + LA < NC)(go)
            else:
                go()
            if g + 1 < NG:
                at_step(c, wq_step, lambda: start_all(wq_descs(g + 1)))
            at_step(c, NC - 1 - LA, lambda: start_all(wo_descs(g)))

        outa = jnp.zeros((G, DM), F32)
        for g in range(NG):
            if g == 0 or NW == 2:
                wait_all(wq_descs(g))
            q = q_group(g) if not dma_only else jnp.zeros((G, DH), BF16)

            def step(c, carry, g=g, q=q):
                m, l, acc = carry
                slot = (g * NC + c) % NS
                issue(g, c)
                b_work(g, c)
                kv_wait(slot)
                if dma_only:
                    return m, l, acc + kvbuf[slot, 0, 0, 0:G, :].astype(F32) + kvbuf[slot, 1, 0, 0:G, :].astype(F32)
                s = None
                for j in range(G):
                    sj = lax.dot_general(q, kvbuf[slot, 0, j], NT, preferred_element_type=F32)
                    s = sj if s is None else jnp.where(row8_r == j, sj, s)
                s = s * SCALE
                m_new = jnp.maximum(m, jnp.max(s, axis=1, keepdims=True))
                alpha = jnp.exp(m - m_new)
                p = jnp.exp(s - m_new)
                l = alpha * l + jnp.sum(p, axis=1, keepdims=True)
                pb = p.astype(BF16)
                pv = None
                for j in range(G):
                    r = jnp.dot(pb, kvbuf[slot, 1, j], preferred_element_type=F32)
                    pv = r if pv is None else jnp.where(row8 == j, r, pv)
                return m_new, l, alpha * acc + pv

            init = (jnp.full((G, 1), -jnp.inf, F32), jnp.zeros((G, 1), F32), jnp.zeros((G, DH), F32))
            if scopes:
                with jax.named_scope("loop%d" % g):
                    m, l, acc = lax.fori_loop(0, NC, step, init)
            else:
                m, l, acc = lax.fori_loop(0, NC, step, init)
            wait_all(wo_descs(g))
            if NW == 1 and g + 1 < NG:
                wait_all(wq_descs(g + 1))
            if dma_only:
                outa = outa + jnp.concatenate([acc] * 4, axis=1)
                continue
            o = (acc / l).astype(BF16).astype(F32)
            for jh in range(HPG):
                h = g + NG * jh
                lhs = jnp.where((row8 == jh) | (row8 == HPG + jh), o, 0.0).astype(BF16)
                outa = outa + jnp.dot(lhs, wo_v[h * DH:(h + 1) * DH, :], preferred_element_type=F32)

        rows = []
        for b in range(NB):
            a = jnp.sum(jnp.where(row8_m // HPG == b, outa, 0.0), axis=0, keepdims=True)
            bb = jnp.sum(outb_s[pl.ds(b * G, G), :], axis=0, keepdims=True)
            rows.append(jnp.concatenate([a, bb], axis=1))
        out_ref[...] = jnp.concatenate(rows, axis=0).astype(out_ref.dtype)

    scratch = [
        pltpu.VMEM((NB, DM), BF16), pltpu.VMEM((NB, DM), BF16),
        pltpu.VMEM((DM, NH * DH), BF16), pltpu.VMEM((NH * DH, DM), BF16),
        pltpu.VMEM((NB, SK, DC), BF16),
        pltpu.VMEM((DM, NH, DH), BF16), pltpu.VMEM((DC, NH, DH), BF16), pltpu.VMEM((DC, NH, DH), BF16),
        pltpu.VMEM((NH, DH, DM), BF16),
        pltpu.VMEM((NS, 2, G, R, DH), BF16),
        pltpu.VMEM((NH, DM, DH), BF16),
        pltpu.VMEM((NH // G, 2 * G, DH), F32), pltpu.VMEM((NH // G, 2 * G, DC), F32),
        pltpu.VMEM((NB, NH, 1), F32), pltpu.VMEM((NB, NH, 1), F32), pltpu.VMEM((NB, NH, DC), F32),
        pltpu.VMEM((NH // G, 2 * G, DH), F32), pltpu.VMEM((2 * G, DM), F32),
        pltpu.SemaphoreType.DMA((NS,)), pltpu.SemaphoreType.DMA((NW + 4,)),
    ]

    def run(A_x, A_k_cache, A_v_cache, A_wq, A_wo, B_x, B_c_kv, B_w_q, B_w_uk, B_w_uv, B_w_o):
        out = pl.pallas_call(
            kernel,
            in_specs=[pl.BlockSpec(memory_space=pl.ANY)] * 11,
            out_specs=pl.BlockSpec(memory_space=pltpu.VMEM),
            out_shape=jax.ShapeDtypeStruct((NB, 2 * DM), BF16),
            scratch_shapes=scratch,
            compiler_params=pltpu.CompilerParams(vmem_limit_bytes=vmem_mb * 2**20, disable_semaphore_checks=nosem, disable_bounds_checks=nobounds),
        )(A_x.reshape(NB, DM), A_k_cache, A_v_cache, A_wq, A_wo,
          B_x.reshape(NB, DM), B_c_kv, B_w_q, B_w_uk, B_w_uv, B_w_o)
        return out.reshape(NB, 1, 2 * DM)
    return run


_RUN = build()


@jax.jit
def pallas_concat_heads__gqa_block_cached__compressed_kv_cla__decode_kernel(
    A_x: jax.Array,
    A_k_cache: jax.Array,
    A_v_cache: jax.Array,
    A_wq: jax.Array,
    A_wo: jax.Array,
    B_x: jax.Array,
    B_c_kv: jax.Array,
    B_w_q: jax.Array,
    B_w_uk: jax.Array,
    B_w_uv: jax.Array,
    B_w_o: jax.Array,
):
    return _RUN(A_x, A_k_cache, A_v_cache, A_wq, A_wo, B_x, B_c_kv, B_w_q, B_w_uk, B_w_uv, B_w_o)
```

```python
import functools

import jax
import jax.numpy as jnp
from jax import lax
from jax.experimental import pallas as pl
from jax.experimental.pallas import tpu as pltpu

F32 = jnp.float32
BF16 = jnp.bfloat16
NT = (((1,), (1,)), ((), ()))

NB, NH, SK, DH = 2, 32, 8192, 128
DM = 512
DC = 512
SCALE = float(DH) ** -0.5

G = 8
HPG = G // NB
NG = NB * NH // G
R = 256
DR = 128
NC = SK // R
NS = 4
LA = NS - 1
W = LA + 1
SIDE = 128
SPS = SIDE // NC
RC = 512
NCH = SK // RC
RL = 64
HP = 4
WQ_STEP = 8

SIDE_PLAN = {0: ("wqb", "wuk"), 1: (("c", 0, 0), ("c", 1, 0)), 2: (("c", 0, 1), ("c", 1, 1)), 3: ("wuv", "wob")}
S_W = 0
SIDE_SEM = {name: 1 + 2 * (g % 2) + w for g, names in SIDE_PLAN.items() for w, name in enumerate(names)}


def _kernel(xa_hbm, k_hbm, v_hbm, wq_hbm, wo_hbm, xb_hbm, c_hbm, wqb_hbm, wuk_hbm, wuv_hbm, wob_hbm,
            out_ref,
            xa_v, xb_v, wq_v, wo_v, c_v, wqb_v, wuk_v, wuv_v, wob_v, kvbuf,
            wt_s, qb_s, qabs_s, mb_s, lb_s, accb_s, ctx_s, outb_s,
            kv_sem, misc_sem):

    def kv_copies(gi, ci, slot):
        out = []
        for d in range(R // DR):
            for j in range(G):
                b, h = j // HPG, gi + NG * (j % HPG)
                for w, src in enumerate((k_hbm, v_hbm)):
                    out.append((pltpu.make_async_copy(src.at[b, h, pl.ds(ci * R + d * DR, DR), :],
                                                      kvbuf.at[slot, w, j, pl.ds(d * DR, DR), :],
                                                      kv_sem.at[slot]), w))
        return out

    head3 = {"wqb": (wqb_hbm, wqb_v), "wuk": (wuk_hbm, wuk_v), "wuv": (wuv_hbm, wuv_v)}

    def side_copy(name, idx):
        if name == "wob":
            r = pl.ds(pl.multiple_of((idx % 4) * 32, 32), 32)
            src, dst = wob_hbm.at[idx // 4, r, :], wob_v.at[idx // 4, r, :]
        elif name in head3:
            r = pl.ds(idx * 4, 4)
            src, dst = head3[name][0].at[r], head3[name][1].at[r]
        else:
            _, b, half = name
            r = pl.ds(half * (SK // 2) + idx * 32, 32)
            src, dst = c_hbm.at[b, r, :], c_v.at[b, r, :]
        return pltpu.make_async_copy(src, dst, misc_sem.at[SIDE_SEM[name]])

    def side_wait(name):
        if name == "wob":
            buf = wob_v
        elif name in head3:
            buf = head3[name][1]
        else:
            _, b, half = name
            buf = c_v.at[b, pl.ds(half * (SK // 2), SK // 2), :]
        pltpu.make_async_copy(buf, buf, misc_sem.at[SIDE_SEM[name]]).wait()

    def wq_copies(g):
        out = []
        for t in range(4):
            for jh in range(HPG):
                r, cc = pl.ds(t * 128, 128), pl.ds((g + NG * jh) * DH, DH)
                out.append((pltpu.make_async_copy(wq_hbm.at[r, cc], wq_v.at[r, cc], misc_sem.at[S_W]), jh % 2))
        return out

    def wo_copies(g):
        out = []
        for t in range(4):
            for jh in range(HPG):
                r = pl.ds((g + NG * jh) * DH + t * 32, 32)
                out.append((pltpu.make_async_copy(wo_hbm.at[r, :], wo_v.at[r, :], misc_sem.at[S_W]), jh % 2))
        return out

    def start_all(copies):
        for cp, queue in copies:
            cp.start(priority=queue)

    def wait_all(copies):
        for cp, _ in copies:
            cp.wait()

    def at_step(c, v, fn):
        pl.when(c == v)(fn)

    row8 = lax.broadcasted_iota(jnp.int32, (G, DH), 0)
    row8_m = lax.broadcasted_iota(jnp.int32, (G, DM), 0)
    row8_r = lax.broadcasted_iota(jnp.int32, (G, R), 0)
    row16_m = lax.broadcasted_iota(jnp.int32, (2 * G, DM), 0)
    row16_d = lax.broadcasted_iota(jnp.int32, (2 * G, DH), 0)

    x_copies = [pltpu.make_async_copy(xa_hbm, xa_v, misc_sem.at[S_W]),
                pltpu.make_async_copy(xb_hbm, xb_v, misc_sem.at[S_W])]
    for cp in x_copies:
        cp.start()
    start_all(wq_copies(0))

    def first_steps(i, carry):
        start_all(kv_copies(0, i, i))
        return carry
    lax.fori_loop(0, LA, first_steps, 0)

    mb_s[...] = jnp.full(mb_s.shape, -jnp.inf, F32)
    for ref in (lb_s, accb_s, qb_s, qabs_s, ctx_s, outb_s):
        ref[...] = jnp.zeros(ref.shape, F32)
    for cp in x_copies:
        cp.wait()
    wait_all(wq_copies(0))

    def keep_rows(rows, jl, x):
        return jnp.where((rows == jl) | (rows == G + jl), x, 0.0).astype(BF16)

    def head_major(w_v, t):
        r = pl.ds(pl.multiple_of(t * RL, RL), RL)
        wt_s[:, r, :] = jnp.swapaxes(w_v[r, :, :], 0, 1)

    def b_query(t):
        x0 = jnp.broadcast_to(xb_v[0:1, :].astype(F32), (2 * G, DM))
        x1 = jnp.broadcast_to(xb_v[1:2, :].astype(F32), (2 * G, DM))
        x01 = jnp.where(row16_m < G, x0, x1)
        hg = HP * t // G
        acc = qb_s[hg]
        for e in range(HP):
            h = HP * t + e
            acc = acc + jnp.dot(keep_rows(row16_m, h % G, x01), wt_s[h], preferred_element_type=F32)
        qb_s[hg] = acc

    def b_absorb(t):
        hg = HP * t // G
        qb = qb_s[hg].astype(BF16).astype(F32)
        acc = qabs_s[hg]
        for e in range(HP):
            h = HP * t + e
            acc = acc + lax.dot_general(keep_rows(row16_d, h % G, qb), wt_s[h], NT, preferred_element_type=F32)
        qabs_s[hg] = acc

    def b_attend(b, ch):
        cc = c_v[b, pl.ds(pl.multiple_of(ch * RC, RC), RC), :]
        qa = jnp.concatenate([qabs_s[hg, pl.ds(pl.multiple_of(b * G, G), G), :] for hg in range(NH // G)],
                             axis=0).astype(BF16)
        s = lax.dot_general(qa, cc, NT, preferred_element_type=F32) * SCALE
        m_prev = mb_s[b]
        m_new = jnp.maximum(m_prev, jnp.max(s, axis=1, keepdims=True))
        alpha = jnp.exp(m_prev - m_new)
        p = jnp.exp(s - m_new)
        lb_s[b] = alpha * lb_s[b] + jnp.sum(p, axis=1, keepdims=True)
        mb_s[b] = m_new
        accb_s[b] = alpha * accb_s[b] + jnp.dot(p.astype(BF16), cc, preferred_element_type=F32)

    def b_context(t):
        hg = HP * t // G
        r0 = pl.ds(pl.multiple_of(hg * G, G), G)
        cc = jnp.concatenate([accb_s[b, r0, :] / lb_s[b, r0, :] for b in range(NB)], axis=0)
        acc = ctx_s[hg]
        for e in range(HP):
            h = HP * t + e
            acc = acc + jnp.dot(keep_rows(row16_m, h % G, cc), wt_s[h], preferred_element_type=F32)
        ctx_s[hg] = acc

    def b_project(t):
        hg = HP * t // G
        ctx = ctx_s[hg].astype(BF16).astype(F32)
        acc = outb_s[...]
        for e in range(HP):
            h = HP * t + e
            acc = acc + jnp.dot(keep_rows(row16_d, h % G, ctx), wob_v[h], preferred_element_type=F32)
        outb_s[...] = acc

    phases = [
        (NC + W, DM // RL, 1, ["wqb"], functools.partial(head_major, wqb_v)),
        (0, NH // HP, 1, [], b_query),
        (0, DC // RL, 1, ["wuk"], functools.partial(head_major, wuk_v)),
        (0, NH // HP, 1, [], b_absorb),
        (2 * NC + W, NB * NCH // 2, 2, [("c", b, 0) for b in range(NB)],
         lambda u: b_attend(u % NB, u // NB)),
        (3 * NC + W, NB * NCH // 2, 2, [("c", b, 1) for b in range(NB)],
         lambda u: b_attend(u % NB, NCH // 2 + u // NB)),
        (4 * NC + W, DC // RL, 1, ["wuv"], functools.partial(head_major, wuv_v)),
        (0, NH // HP, 1, [], b_context),
        (0, NH // HP, 1, ["wob"], b_project),
    ]
    started_in = {name: g for g, names in SIDE_PLAN.items() for name in names}
    plan, end = [], 0
    for lo, n, stride, names, fn in phases:
        lo = max(lo, end)
        end = lo + n * stride
        for name in names:
            g0 = started_in[name]
            assert lo >= (g0 + 1) * NC + W and (g0 + 2 not in SIDE_PLAN or lo < (g0 + 2) * NC)
        plan.append((lo, end, stride, names, fn))
    assert end <= NG * NC

    def b_work(g, c):
        for lo, hi, stride, names, fn in plan:
            if names and lo // NC == g:
                @pl.when(c == lo % NC)
                def _(names=names):
                    for name in names:
                        side_wait(name)
            a, z = max(lo, g * NC), min(hi, (g + 1) * NC)
            if a < z:
                i = c + (g * NC - lo)
                cond = (c >= a - g * NC) & (c < z - g * NC)
                if stride > 1:
                    cond = cond & (i % stride == 0)
                pl.when(cond)(functools.partial(fn, i // stride))

    def issue(g, c):
        nxt = g * NC + c + LA

        def go():
            kv = kv_copies(nxt // NC, nxt % NC, nxt % NS)
            if g not in SIDE_PLAN:
                start_all(kv)
                return
            n = len(kv) // SPS
            for t in range(SPS):
                start_all(kv[n * t:n * (t + 1)])
                for queue, name in enumerate(SIDE_PLAN[g]):
                    side_copy(name, c + NC * t).start(priority=queue)

        if g == NG - 1:
            pl.when(c + LA < NC)(go)
        else:
            go()
            at_step(c, WQ_STEP, lambda: start_all(wq_copies(g + 1)))
        at_step(c, NC - 1 - LA, lambda: start_all(wo_copies(g)))

    x0 = jnp.broadcast_to(xa_v[0:1, :].astype(F32), (G, DM))
    x1 = jnp.broadcast_to(xa_v[1:2, :].astype(F32), (G, DM))
    outa = jnp.zeros((G, DM), F32)
    for g in range(NG):
        q = jnp.zeros((G, DH), F32)
        for jh in range(HPG):
            h = g + NG * jh
            lhs = jnp.where(row8_m == jh, x0, jnp.where(row8_m == HPG + jh, x1, 0.0)).astype(BF16)
            q = q + jnp.dot(lhs, wq_v[:, h * DH:(h + 1) * DH], preferred_element_type=F32)
        q = q.astype(BF16)

        def step(c, carry, g=g, q=q):
            m, l, acc = carry
            slot = (g * NC + c) % NS
            issue(g, c)
            b_work(g, c)
            pltpu.make_async_copy(kvbuf.at[slot], kvbuf.at[slot], kv_sem.at[slot]).wait()
            s = None
            for j in range(G):
                sj = lax.dot_general(q, kvbuf[slot, 0, j], NT, preferred_element_type=F32)
                s = sj if s is None else jnp.where(row8_r == j, sj, s)
            s = s * SCALE
            m_new = jnp.maximum(m, jnp.max(s, axis=1, keepdims=True))
            alpha = jnp.exp(m - m_new)
            p = jnp.exp(s - m_new)
            l = alpha * l + jnp.sum(p, axis=1, keepdims=True)
            pb = p.astype(BF16)
            pv = None
            for j in range(G):
                r = jnp.dot(pb, kvbuf[slot, 1, j], preferred_element_type=F32)
                pv = r if pv is None else jnp.where(row8 == j, r, pv)
            return m_new, l, alpha * acc + pv

        init = (jnp.full((G, 1), -jnp.inf, F32), jnp.zeros((G, 1), F32), jnp.zeros((G, DH), F32))
        _, l, acc = lax.fori_loop(0, NC, step, init)
        wait_all(wo_copies(g))
        if g + 1 < NG:
            wait_all(wq_copies(g + 1))
        o = (acc / l).astype(BF16).astype(F32)
        for jh in range(HPG):
            h = g + NG * jh
            lhs = jnp.where((row8 == jh) | (row8 == HPG + jh), o, 0.0).astype(BF16)
            outa = outa + jnp.dot(lhs, wo_v[h * DH:(h + 1) * DH, :], preferred_element_type=F32)

    rows = []
    for b in range(NB):
        a = jnp.sum(jnp.where(row8_m // HPG == b, outa, 0.0), axis=0, keepdims=True)
        bb = jnp.sum(outb_s[pl.ds(b * G, G), :], axis=0, keepdims=True)
        rows.append(jnp.concatenate([a, bb], axis=1))
    out_ref[...] = jnp.concatenate(rows, axis=0).astype(out_ref.dtype)


@jax.jit
def pallas_concat_heads__gqa_block_cached__compressed_kv_cla__decode_kernel(
    A_x: jax.Array,
    A_k_cache: jax.Array,
    A_v_cache: jax.Array,
    A_wq: jax.Array,
    A_wo: jax.Array,
    B_x: jax.Array,
    B_c_kv: jax.Array,
    B_w_q: jax.Array,
    B_w_uk: jax.Array,
    B_w_uv: jax.Array,
    B_w_o: jax.Array,
):
    scratch = [
        pltpu.VMEM((NB, DM), BF16), pltpu.VMEM((NB, DM), BF16),
        pltpu.VMEM((DM, NH * DH), BF16), pltpu.VMEM((NH * DH, DM), BF16),
        pltpu.VMEM((NB, SK, DC), BF16),
        pltpu.VMEM((DM, NH, DH), BF16), pltpu.VMEM((DC, NH, DH), BF16),
        pltpu.VMEM((DC, NH, DH), BF16), pltpu.VMEM((NH, DH, DM), BF16),
        pltpu.VMEM((NS, 2, G, R, DH), BF16),
        pltpu.VMEM((NH, DM, DH), BF16),
        pltpu.VMEM((NH // G, 2 * G, DH), F32), pltpu.VMEM((NH // G, 2 * G, DC), F32),
        pltpu.VMEM((NB, NH, 1), F32), pltpu.VMEM((NB, NH, 1), F32),
        pltpu.VMEM((NB, NH, DC), F32),
        pltpu.VMEM((NH // G, 2 * G, DH), F32), pltpu.VMEM((2 * G, DM), F32),
        pltpu.SemaphoreType.DMA((NS,)), pltpu.SemaphoreType.DMA((5,)),
    ]
    out = pl.pallas_call(
        _kernel,
        in_specs=[pl.BlockSpec(memory_space=pl.ANY)] * 11,
        out_specs=pl.BlockSpec(memory_space=pltpu.VMEM),
        out_shape=jax.ShapeDtypeStruct((NB, 2 * DM), BF16),
        scratch_shapes=scratch,
        compiler_params=pltpu.CompilerParams(vmem_limit_bytes=100 * 2**20),
    )(A_x.reshape(NB, DM), A_k_cache, A_v_cache, A_wq, A_wo,
      B_x.reshape(NB, DM), B_c_kv, B_w_q, B_w_uk, B_w_uv, B_w_o)
    return out.reshape(NB, 1, 2 * DM)
```
